```python
import os as _os
_os.environ.setdefault("JAX_PLATFORMS", "cpu")
import jax
import jax.numpy as jnp

def _softmax(x, axis=-1):
    return jax.nn.softmax(x, axis=axis)
def _gelu(x):
    return jax.nn.gelu(x, approximate=True)
def _silu(x):
    return jax.nn.silu(x)
def _sigmoid(x):
    return jax.nn.sigmoid(x)
def _layernorm(x, axis=-1, eps=1e-5):
    m = jnp.mean(x, axis=axis, keepdims=True)
    v = jnp.var(x, axis=axis, keepdims=True)
    return (x - m) / jnp.sqrt(v + eps)
def _scatter_add(tgt, idx, src, axis=0):
    return tgt.at[idx].add(src)
def _segment_sum(src, seg, n):
    return jax.ops.segment_sum(src, seg, n)
class _Rng:
    def __init__(self, key):
        self._k = key
    def _next(self):
        self._k, sub = jax.random.split(self._k)
        return sub
    def normal(self, shape):
        return jax.random.normal(self._next(), shape, dtype=jnp.bfloat16)
    def randint(self, lo, hi, shape):
        return jax.random.randint(self._next(), shape, lo, hi, dtype=jnp.int32)
    def uniform(self, shape, lo=0.0, hi=1.0):
        return jax.random.uniform(self._next(), shape, jnp.bfloat16, lo, hi)
    def permutation(self, n):
        return jax.random.permutation(self._next(), n)


kernel_name = 'sequential_preLN__mha_block__swiglu_ffn__prompt'

def setup_inputs():
    _rng = _Rng(jax.random.key(int.from_bytes(__import__("os").urandom(4), "little")))
    _w = (lambda a: (lambda t: t.astype(jnp.bfloat16) if jnp.issubdtype(t.dtype, jnp.floating) else t)(jnp.asarray(a)))
    def _A_setup():
        B, S, D, H = 1, 2048, 640, 32
        return {
            "x": _w((lambda *s: _rng.normal(s) * 0.05)(B, S, D)),
            "wqkv": _w((lambda *s: _rng.normal(s) * 0.05)(D, 3 * D)),
            "wo": _w((lambda *s: _rng.normal(s) * 0.05)(D, D)),
        }
    _A_in = _A_setup()

    def _B_setup():
        B, S, D, F = 1, 2048, 640, 1728
        return {
            "x": _w((lambda *s: _rng.normal(s) * 0.05)(B, S, D)),
            "w_gate": _w((lambda *s: _rng.normal(s) * 0.05)(D, F)),
            "w_up": _w((lambda *s: _rng.normal(s) * 0.05)(D, F)),
            "w_down": _w((lambda *s: _rng.normal(s) * 0.05)(F, D)),
        }
    _B_in = _B_setup()

    return {
        "A_x": _A_in["x"],
        "A_wqkv": _A_in["wqkv"],
        "A_wo": _A_in["wo"],
        "B_x": _B_in["x"],
        "B_w_gate": _B_in["w_gate"],
        "B_w_up": _B_in["w_up"],
        "B_w_down": _B_in["w_down"],
    }

def reference(A_x, A_wqkv, A_wo, B_x, B_w_gate, B_w_up, B_w_down):
    def _A_ref(x, wqkv, wo):
        B, S, D = x.shape
        H = 32
        Dh = D // H
        qkv = (lambda x, *d: x.transpose(*d))((x @ wqkv).reshape(B, S, 3, H, Dh), 2, 0, 3, 1, 4)
        q, k, v = qkv[0], qkv[1], qkv[2]
        scores = jnp.einsum("bhqd,bhkd->bhqk", q, k) * (Dh ** -0.5)
        p = _softmax(scores, axis=-1)
        o = jnp.einsum("bhqk,bhkd->bhqd", p, v)
        return (lambda x, *d: x.transpose(*d))(o, 0, 2, 1, 3).reshape(B, S, D) @ wo

    def _B_ref(x, w_gate, w_up, w_down):
        g = _silu(x @ w_gate)
        u = x @ w_up
        return (g * u) @ w_down

    x = A_x
    h = x + _A_ref(_layernorm(x, axis=-1), A_wqkv, A_wo)
    h2 = h + _B_ref(_layernorm(h, axis=-1), B_w_gate, B_w_up, B_w_down)
    return h2
```

```python
import math

import jax
import jax.numpy as jnp
from jax import lax
import jax.experimental.pallas as pl
import jax.experimental.pallas.tpu as pltpu

S, D, H, DH, F = 2048, 640, 32, 20, 1728
TQ = 512
CK = 128
PC = 256
FC = 256
UH = 8
KW = 32
VR = 24
NC = S // CK
NP = S // PC
GMAX = (S // TQ) * H - 1
FM = F // 128 * 128
FR = F - FM
BF = jnp.bfloat16
F32 = jnp.float32
QSCALE = (DH ** -0.5) * math.log2(math.e)
NN = (((1,), (0,)), ((), ()))
NT = (((1,), (1,)), ((), ()))
TN = (((0,), (0,)), ((), ()))


def _dot(a, b, dims):
    return lax.dot_general(a, b, dims, preferred_element_type=F32)


def _ln(x):
    m = jnp.mean(x, axis=-1, keepdims=True)
    xc = x - m
    v = jnp.mean(xc * xc, axis=-1, keepdims=True)
    return xc * lax.rsqrt(v + 1e-5)


def _kernel(x_hbm, wqkv_hbm, wo_hbm, wgt_hbm, wut_hbm, wd_hbm, o_ref,
            x_ref, wqkv_ref, wo_ref, wgt_ref, wut_ref, wd_ref, wgu_ref,
            wt_ref, xn_ref, qt_ref, k_ref, vt_ref, s_ref, at_ref, mx_ref, qm0_ref, qm1_ref,
            hres_ref, xsem, wsem):
    i = pl.program_id(0)
    qm_refs = (qm0_ref, qm1_ref)

    def x_copy(c):
        r = pl.multiple_of(c * PC, PC)
        return pltpu.make_async_copy(x_hbm.at[pl.ds(r, PC)], x_ref.at[pl.ds(r, PC)], xsem.at[c])

    def wqkv_copy(n):
        cols = slice(n * D, (n + 1) * D)
        return pltpu.make_async_copy(wqkv_hbm.at[:, cols], wqkv_ref.at[:, cols], wsem.at[n])

    late = [pltpu.make_async_copy(a, b, wsem.at[3 + n]) for n, (a, b) in enumerate(
        [(wo_hbm, wo_ref), (wgt_hbm, wgt_ref), (wut_hbm, wut_ref), (wd_hbm, wd_ref)])]

    def make_qm(g, slot):
        g = jnp.minimum(g, GMAX)
        blk = g // H
        h = g - blk * H
        a = pl.multiple_of(h * DH // 8 * 8, 8)
        row = lax.broadcasted_iota(jnp.int32, (KW, TQ), 0) + (a - h * DH)
        qs = qt_ref[pl.ds(a, KW), pl.ds(pl.multiple_of(blk * TQ, TQ), TQ)]
        qm_refs[slot][...] = jnp.where((row >= 0) & (row < DH), qs, 0.0).astype(BF)
        return h

    def qk(c, h, qm, slot, mx):
        ks = slice(c * CK, (c + 1) * CK)
        s = _dot(k_ref[h, ks, :], qm, NN)
        s_ref[slot, ks, :] = s
        cm = jnp.max(s.reshape(CK // 8, 8, TQ), axis=0)
        return cm if mx is None else jnp.maximum(mx, cm)

    def stage(g, h, slot, mx_cur, mx_next, h_next, qm):
        a = pl.multiple_of(h * DH // 8 * 8, 8)
        off = h * DH - a
        onerow = jnp.where(off == 0, VR - 1, 0)
        vrow = lax.broadcasted_iota(jnp.int32, (VR, CK), 0)
        m = jnp.max(mx_cur, axis=0, keepdims=True)
        o = None
        for c in range(NC):
            if c + 1 < NC:
                mx_next = qk(c + 1, h_next, qm, 1 - slot, mx_next)
            else:
                qm = qm_refs[slot][...]
                mx_next2 = qk(0, h_next2, qm, slot, None)
            ks = slice(c * CK, (c + 1) * CK)
            p = jnp.exp2(s_ref[slot, ks, :] - m).astype(BF)
            vw = jnp.where(vrow == onerow, 1.0, vt_ref[pl.ds(a, VR), ks])
            oc = _dot(vw, p, NN)
            o = oc if o is None else o + oc
            if c == 4:
                h_next2 = make_qm(g + 2, slot)
        row = lax.broadcasted_iota(jnp.int32, (VR, TQ), 0)
        l = jnp.sum(jnp.where(row == onerow, o, 0.0), axis=0, keepdims=True)
        old = at_ref[pl.ds(a, VR), :]
        at_ref[pl.ds(a, VR), :] = jnp.where((row >= off) & (row < off + DH), o * (1.0 / l), old)
        return mx_next, mx_next2, h_next2, qm

    @pl.when(i == 0)
    def _prologue():
        wqkv_copy(0).start()
        x_copy(0).start()
        wqkv_copy(1).start()
        wqkv_copy(2).start()
        at_ref[...] = jnp.zeros((D, TQ), F32)
        qt_ref[D:, :] = jnp.zeros((8, S), F32)
        for n in range(3):
            wqkv_copy(n).wait()
            if n == 0:
                for c in range(1, NP):
                    x_copy(c).start()
            if n == 1:
                x_copy(0).wait()
                xn_ref[...] = _ln(x_ref[:PC, :].astype(F32)).astype(BF)
            if n == 2:
                for cp in late:
                    cp.start()
            wt_ref[n * D:(n + 1) * D, :] = wqkv_ref[:, n * D:(n + 1) * D].T

        def project(c, _):
            r = pl.multiple_of(c * PC, PC)
            cn = jnp.minimum(c + 1, NP - 1)

            @pl.when(c + 1 < NP)
            def _():
                x_copy(cn).wait()
            xn = xn_ref[...]
            kt = _dot(wt_ref[D:2 * D, :], xn, NT)
            kt = jnp.concatenate([kt, jnp.zeros((8, PC), F32)], axis=0)
            for h in range(H):
                a = h * DH // 8 * 8
                k_ref[h, pl.ds(r, PC), :] = kt[a:a + KW].astype(BF).T
            qt_ref[:D, pl.ds(r, PC)] = _dot(wt_ref[:D, :], xn, NT) * QSCALE
            xn_ref[...] = _ln(x_ref[pl.ds(pl.multiple_of(cn * PC, PC), PC), :].astype(F32)).astype(BF)
            vt_ref[:, pl.ds(r, PC)] = _dot(wt_ref[2 * D:, :], xn, NT).astype(BF).astype(F32)
            return 0
        lax.fori_loop(0, NP, project, 0)

        make_qm(0, 0)
        make_qm(1, 1)
        for h, n in ((0, NC), (1, 1)):
            mx, qm = None, qm_refs[h][...]
            for c in range(n):
                mx = qk(c, h, qm, h, mx)
            mx_ref[h] = mx

    def heads(t, carry):
        carry = carry + (qm1_ref[...],)
        for u in range(UH):
            h = UH * t + u
            carry = stage(i * H + h, h, u % 2, *carry)
        return carry[:3]
    mx_ref[0], mx_ref[1], _ = lax.fori_loop(0, H // UH, heads, (mx_ref[0], mx_ref[1], 1))

    @pl.when(i == 0)
    def _():
        for cp in late:
            cp.wait()
        wgu_ref[:FR, :] = wgt_ref[FM:, :]
        wgu_ref[FR:, :] = wut_ref[FM:, :]

    q0 = pl.multiple_of(i * TQ, TQ)

    def norm(c, attn):
        hres = x_ref[pl.ds(q0 + c * FC, FC), :].astype(F32) + attn
        hres_ref[c * FC:(c + 1) * FC, :] = hres
        return _ln(hres).astype(BF)

    nf = TQ // FC
    attn = [_dot(at_ref[:, c * FC:(c + 1) * FC].astype(BF), wo_ref[...], TN) for c in range(nf)]
    hn = norm(0, attn[0])
    for c in range(nf):
        rs = slice(c * FC, (c + 1) * FC)
        gu = _dot(hn, wgu_ref[...], NT)
        g = _dot(hn, wgt_ref[:FM, :], NT)
        u = _dot(hn, wut_ref[:FM, :], NT)
        act = (g * jax.nn.sigmoid(g) * u).astype(BF)
        act2 = (gu * jax.nn.sigmoid(gu) * pltpu.roll(gu, FR, 1))[:, :FR].astype(BF)
        if c + 1 < nf:
            hn = norm(c + 1, attn[c + 1])
        y = _dot(act2, wd_ref[FM:, :], NN) + _dot(act, wd_ref[:FM, :], NN)
        o_ref[rs, :] = (hres_ref[rs, :] + y).astype(o_ref.dtype)


@jax.jit
def pallas_sequential_preLN__mha_block__swiglu_ffn__prompt_kernel(
    A_x: jax.Array,
    A_wqkv: jax.Array,
    A_wo: jax.Array,
    B_x: jax.Array,
    B_w_gate: jax.Array,
    B_w_up: jax.Array,
    B_w_down: jax.Array,
):
    del B_x
    out = pl.pallas_call(
        _kernel,
        grid=(S // TQ,),
        in_specs=[pl.BlockSpec(memory_space=pl.ANY)] * 6,
        out_specs=pl.BlockSpec((TQ, D), lambda i: (i, 0)),
        out_shape=jax.ShapeDtypeStruct((S, D), A_x.dtype),
        scratch_shapes=[
            pltpu.VMEM((S, D), BF),
            pltpu.VMEM((D, 3 * D), BF),
            pltpu.VMEM((D, D), BF),
            pltpu.VMEM((F, D), BF),
            pltpu.VMEM((F, D), BF),
            pltpu.VMEM((F, D), BF),
            pltpu.VMEM((2 * FR, D), BF),
            pltpu.VMEM((3 * D, D), BF),
            pltpu.VMEM((PC, D), BF),
            pltpu.VMEM((D + 8, S), F32),
            pltpu.VMEM((H, S, KW), BF),
            pltpu.VMEM((D, S), F32),
            pltpu.VMEM((2, S, TQ), F32),
            pltpu.VMEM((D, TQ), F32),
            pltpu.VMEM((2, 8, TQ), F32),
            pltpu.VMEM((KW, TQ), BF),
            pltpu.VMEM((KW, TQ), BF),
            pltpu.VMEM((TQ, D), F32),
            pltpu.SemaphoreType.DMA((NP,)),
            pltpu.SemaphoreType.DMA((7,)),
        ],
        compiler_params=pltpu.CompilerParams(
            dimension_semantics=("arbitrary",), vmem_limit_bytes=100 * 2**20),
        name="mha_ffn",
    )(A_x.reshape(S, D), A_wqkv, A_wo, B_w_gate.T, B_w_up.T, B_w_down)
    return out.reshape(1, S, D)
```
